```python
import os as _os
_os.environ.setdefault("JAX_PLATFORMS", "cpu")
import jax
import jax.numpy as jnp

def _softmax(x, axis=-1):
    return jax.nn.softmax(x, axis=axis)
def _gelu(x):
    return jax.nn.gelu(x, approximate=True)
def _silu(x):
    return jax.nn.silu(x)
def _sigmoid(x):
    return jax.nn.sigmoid(x)
def _layernorm(x, axis=-1, eps=1e-5):
    m = jnp.mean(x, axis=axis, keepdims=True)
    v = jnp.var(x, axis=axis, keepdims=True)
    return (x - m) / jnp.sqrt(v + eps)
def _scatter_add(tgt, idx, src, axis=0):
    return tgt.at[idx].add(src)
def _segment_sum(src, seg, n):
    return jax.ops.segment_sum(src, seg, n)
class _Rng:
    def __init__(self, key):
        self._k = key
    def _next(self):
        self._k, sub = jax.random.split(self._k)
        return sub
    def normal(self, shape):
        return jax.random.normal(self._next(), shape, dtype=jnp.bfloat16)
    def randint(self, lo, hi, shape):
        return jax.random.randint(self._next(), shape, lo, hi, dtype=jnp.int32)
    def uniform(self, shape, lo=0.0, hi=1.0):
        return jax.random.uniform(self._next(), shape, jnp.bfloat16, lo, hi)
    def permutation(self, n):
        return jax.random.permutation(self._next(), n)


kernel_name = 'interleave_layers__sliding_block_cached__mixer_channel_mlp__decode'

def setup_inputs():
    _rng = _Rng(jax.random.key(int.from_bytes(__import__("os").urandom(4), "little")))
    _w = (lambda a: (lambda t: t.astype(jnp.bfloat16) if jnp.issubdtype(t.dtype, jnp.floating) else t)(jnp.asarray(a)))
    def _A_setup():
        B, Sq, D = 8, 1, 1024
        Hq, Hkv, Sk, Dh = 32, 4, 4096, 128
        assert Hq % Hkv == 0, (Hq, Hkv)
        return {
            "x": _w((lambda *s: _rng.normal(s) * 0.05)(B, Sq, D)),
            "k_cache": _w((lambda *s: _rng.normal(s) * 1.6)(B, Hkv, Sk, Dh)),
            "v_cache": _w((lambda *s: _rng.normal(s) * 0.8)(B, Hkv, Sk, Dh)),
            "wq": _w((lambda *s: _rng.normal(s) * 1.6)(D, Hq * Dh) * (D ** -0.5)),
            "wo": _w((lambda *s: _rng.normal(s) * 0.8)(Hq * Dh, D) * ((Hq * Dh) ** -0.5)),
        }
    _A_in = _A_setup()

    def _B_setup():
        B, S, D, F = 8, 1, 1024, 3584
        return {
            "x": _w((lambda *s: _rng.normal(s) * 0.05)(B, S, D)),
            "w1": _w((lambda *s: _rng.normal(s) * 0.4)(D, F) * (D ** -0.5)),
            "b1": _w((lambda *s: _rng.normal(s) * 0.4)(F)),
            "w2": _w((lambda *s: _rng.normal(s) * 0.4)(F, D) * (F ** -0.5)),
            "b2": _w((lambda *s: _rng.normal(s) * 0.1)(D)),
        }
    _B_in = _B_setup()

    return {
        "A_x": _A_in["x"],
        "A_k_cache": _A_in["k_cache"],
        "A_v_cache": _A_in["v_cache"],
        "A_wq": _A_in["wq"],
        "A_wo": _A_in["wo"],
        "B_x": _B_in["x"],
        "B_w1": _B_in["w1"],
        "B_b1": _B_in["b1"],
        "B_w2": _B_in["w2"],
        "B_b2": _B_in["b2"],
    }

def reference(A_x, A_k_cache, A_v_cache, A_wq, A_wo, B_x, B_w1, B_b1, B_w2, B_b2):
    def _A_ref(x, k_cache, v_cache, wq, wo):
        B, Sq, D = x.shape
        Hq, Dh = 32, 128
        Hkv, Sk = k_cache.shape[1], k_cache.shape[2]
        W = min(4096, max(256, Sk // 4))
        rep = Hq // Hkv
        q = (lambda x, *d: x.transpose(*d))((x @ wq).reshape(B, Sq, Hq, Dh), 0, 2, 1, 3)
        k = jnp.repeat(k_cache[:, :, Sk - W:, :], rep, axis=1)
        v = jnp.repeat(v_cache[:, :, Sk - W:, :], rep, axis=1)
        scores = jnp.einsum("bhqd,bhkd->bhqk", q, k) * (Dh ** -0.5)
        p = _softmax(scores, axis=-1)
        o = jnp.einsum("bhqk,bhkd->bhqd", p, v)
        return (lambda x, *d: x.transpose(*d))(o, 0, 2, 1, 3).reshape(B, Sq, Hq * Dh) @ wo

    def _B_ref(x, w1, b1, w2, b2):
        y = _layernorm(x, axis=-1)
        h = _gelu(jnp.einsum("bsd,df->bsf", y, w1) + b1)
        return jnp.einsum("bsf,fd->bsd", h, w2) + b2

    x = A_x
    x = x + _A_ref(_layernorm(x, axis=-1), A_k_cache, A_v_cache, A_wq, A_wo)
    x = x + _B_ref(_layernorm(x, axis=-1), B_w1, B_b1, B_w2, B_b2)
    x = x + _A_ref(_layernorm(x, axis=-1), A_k_cache, A_v_cache, A_wq, A_wo)
    x = x + _B_ref(_layernorm(x, axis=-1), B_w1, B_b1, B_w2, B_b2)
    return x
```

```python
import jax
import jax.numpy as jnp
from jax import lax
import jax.experimental.pallas as pl
import jax.experimental.pallas.tpu as pltpu

_EPS = 1e-5
_L = 128


def _gelu_tanh(x):
    c = 0.7978845608028654
    return 0.5 * x * (1.0 + jnp.tanh(c * (x + 0.044715 * (x * x * x))))


def _dot(a, b):
    return jnp.dot(a, b, preferred_element_type=jnp.float32)


def _ln_stats(x):
    m = jnp.mean(x, axis=-1, keepdims=True)
    xc = x - m
    v = jnp.mean(xc * xc, axis=-1, keepdims=True)
    return m, lax.rsqrt(v + _EPS), xc


def _interleave(lists):
    out = []
    for tup in zip(*lists):
        out.extend(tup)
    return out


def _pieces_2d(h, v, r0, nrows, c0, ncols, ns, pr, pc):
    per = nrows // ns
    assert per * ns == nrows and per % pr == 0 and ncols % pc == 0
    return _interleave([
        [(h.at[pl.ds(r, pr), pl.ds(c0 + c, pc)], v.at[pl.ds(r, pr), pl.ds(c, pc)])
         for r in range(r0 + s * per, r0 + (s + 1) * per, pr) for c in range(0, ncols, pc)]
        for s in range(ns)])


CFG = dict(LA=96, LAG=4, LAG2=4, NE=4, PUMP=1)


@jax.jit
def pallas_interleave_layers__sliding_block_cached__mixer_channel_mlp__decode_kernel(
        A_x, A_k_cache, A_v_cache, A_wq, A_wo, B_x, B_w1, B_b1, B_w2, B_b2):
    B, Sq, D = A_x.shape
    _, Hkv, Sk, Dh = A_k_cache.shape
    Hq = A_wq.shape[1] // Dh
    F = B_w1.shape[1]
    W = min(4096, max(256, Sk // 4))
    rep = Hq // Hkv
    scale = Dh ** -0.5
    bf16 = jnp.bfloat16
    f32 = jnp.float32
    ND, NF, NW = D // _L, F // _L, W // _L
    HD = Hq * Dh
    CA, CB, CC = 5, 2, 1
    assert CA + CB + CC == ND
    FC1 = NF - 4
    LA, LAG, LAG2, NE = CFG["LA"], CFG["LAG"], CFG["LAG2"], CFG["NE"]
    NSEM = 3
    pairs = [(g, b) for g in range(Hkv) for b in range(B)]

    def kernel(x_h, k_h, v_h, wq_h, wo_h, w1_h, b1_h, w2_h, b2_h, o_ref,
               x_v, b1_v, b2_v, wq_v, k_v, v_v, wo_v, w1_v, w2a_v, w2b_v, w2c_v,
               kt_r, q_s, o_s, csq_s, cs1_s, b1_s, qp_s, sems):
        tasks = []
        tasks.append(([(x_h, x_v), (b1_h, b1_v), (b2_h, b2_v)]
                      + _pieces_2d(wq_h, wq_v, 0, D, 0, HD, 8, 8, HD // 2),
                      [x_v, b1_v, b2_v, wq_v]))
        for b in range(B):
            tasks.append(([(c_h.at[b, g, pl.ds(Sk - W + r, _L), :], c_v.at[b, g, pl.ds(r, _L), :])
                           for r in range(0, W, _L) for g in range(Hkv)
                           for c_h, c_v in ((k_h, k_v), (v_h, v_v))],
                          [k_v.at[b], v_v.at[b]]))
        tasks.append((_pieces_2d(wo_h, wo_v, 0, HD, 0, D, 8, 16, D), [wo_v]))
        tasks.append((_pieces_2d(w1_h, w1_v, 0, D, 0, F, 8, 8, F // 2), [w1_v]))
        tasks.append((_pieces_2d(w2_h, w2a_v, 0, F, 0, CA * _L, 8, 32, CA * _L), [w2a_v]))
        tasks.append((_pieces_2d(w2_h, w2b_v, 0, F, CA * _L, CB * _L, 8, 64, CB * _L), [w2b_v]))
        tasks.append((_pieces_2d(w2_h, w2c_v, 0, FC1 * _L, (CA + CB) * _L, CC * _L, 8, 64, CC * _L),
                      [w2c_v.at[pl.ds(0, FC1 * _L)]]))
        tasks.append((_pieces_2d(w2_h, w2c_v, FC1 * _L, F - FC1 * _L, (CA + CB) * _L, CC * _L, 8, 64, CC * _L),
                      [w2c_v.at[pl.ds(FC1 * _L, F - FC1 * _L)]]))
        flat = [(s, d, t) for t, (ps, _) in enumerate(tasks) for s, d in ps]
        ends = []
        for ps, _ in tasks:
            ends.append((ends[-1] if ends else 0) + len(ps))
        state = dict(issued=0, waited=0)

        def issue_until(n):
            n = min(n, len(flat))
            while state["issued"] < n:
                i = state["issued"]
                s, d, t = flat[i]
                assert t < state["waited"] + NSEM
                pltpu.make_async_copy(s, d, sems.at[t % NSEM]).start(priority=i % 2)
                state["issued"] += 1

        def pump(k):
            t = state["waited"]
            cap = ends[t] + LA if t < len(tasks) else len(flat)
            lim = ends[min(t + NSEM - 1, len(tasks) - 1)]
            issue_until(min(state["issued"] + k * CFG["PUMP"], cap, lim))

        def wait_task(t):
            assert t == state["waited"]
            issue_until(min(ends[t] + LA, ends[min(t + NSEM - 1, len(tasks) - 1)]))
            for buf in tasks[t][1]:
                pltpu.make_async_copy(buf, buf, sems.at[t % NSEM]).wait()
            state["waited"] += 1

        ones = jnp.ones((B, D), bf16)

        def rowblocks(lhs, w_ref, k0, k1, acc=None):
            for k in range(k0, k1):
                r = _dot(lhs[:, (k - k0) * _L:(k - k0 + 1) * _L], w_ref[k * _L:(k + 1) * _L, :])
                acc = r if acc is None else acc + r
                pump(max(1, w_ref.shape[1] // (8 * _L)))
            return acc

        wait_task(0)
        x = x_v[...].astype(f32)
        b1_s[...] = jnp.broadcast_to(b1_v[...].astype(f32).reshape(1, F), (B, F))
        b2 = jnp.broadcast_to(b2_v[...].astype(f32).reshape(1, D), (B, D))
        _, r, xc = _ln_stats(x)
        lhs = jnp.concatenate([(xc * r).astype(bf16), ones], axis=0)
        QC = 8 * _L
        for c in range(0, HD, QC):
            res = rowblocks(lhs, wq_v.at[:, pl.ds(c, QC)], 0, ND)
            csq_s[:, c:c + QC] = res[B:]
            for h in range(c // _L, (c + QC) // _L):
                q_s[h * B:(h + 1) * B, :] = res[:B, h * _L - c:(h + 1) * _L - c] * scale

        for b in range(B):
            wait_task(1 + b)

            for g in range(Hkv):
                rows = pl.ds(g * rep * B + b, rep, stride=B)
                qbg = q_s[rows, :].astype(bf16)
                ss = []
                for t in range(NW):
                    kt = k_v[b, g, t * _L:(t + 1) * _L, :].T
                    kt_r[(g * B + b) * NW + t] = kt
                    ss.append(_dot(qbg, kt))
                    pump(2)
                s = jnp.concatenate(ss, axis=1)
                m = jnp.max(s, axis=-1, keepdims=True)
                p = jnp.exp(s - m)
                l = jnp.sum(p, axis=-1, keepdims=True)
                o_s[rows, :] = _dot(p.astype(bf16), v_v[b, g]) / l

        oc = jnp.concatenate([o_s[h * B:(h + 1) * B, :] for h in range(Hq)], axis=1).astype(bf16)
        wait_task(1 + B)
        x = rowblocks(oc, wo_v, 0, Hq, x).astype(bf16).astype(f32)
        _, r, xc = _ln_stats(x)
        _, r2, uc = _ln_stats(xc * r)
        lhs = jnp.concatenate([(uc * r2).astype(bf16), ones], axis=0)

        wait_task(2 + B)
        hs = []
        for f in range(NF):
            res = _dot(lhs, w1_v[:, f * _L:(f + 1) * _L])
            cs1_s[:, f * _L:(f + 1) * _L] = res[B:]
            hs.append(_gelu_tanh(res[:B] + b1_s[:, f * _L:(f + 1) * _L]).astype(bf16))
            pump(1)
        hc = jnp.concatenate(hs, axis=1)
        xb2 = x + b2

        wait_task(3 + B)
        xa = rowblocks(hc, w2a_v, 0, NF, xb2[:, :CA * _L]).astype(bf16)
        for c in range(0, HD, QC):
            qp_s[:, c:c + QC] = rowblocks(xa, wq_v.at[:, pl.ds(c, QC)], 0, CA)
        wait_task(4 + B)
        xbb = (xb2[:, CA * _L:(CA + CB) * _L] + _dot(hc, w2b_v[...])).astype(bf16)
        for c in range(0, HD, QC):
            qp_s[:, c:c + QC] = rowblocks(xbb, wq_v.at[:, pl.ds(c, QC)], CA, CA + CB, qp_s[:, c:c + QC])
        wait_task(5 + B)
        xcc = xb2[:, (CA + CB) * _L:] + _dot(hc[:, :FC1 * _L], w2c_v[0:FC1 * _L, :])
        wait_task(6 + B)
        xcc = (xcc + _dot(hc[:, FC1 * _L:], w2c_v[FC1 * _L:, :])).astype(bf16)

        x = jnp.concatenate([xa, xbb, xcc], axis=1).astype(f32)
        m, r, _ = _ln_stats(x)
        rs = r * scale
        for c in range(0, HD, QC):
            raw = rowblocks(xcc, wq_v.at[:, pl.ds(c, QC)], CA + CB, ND, qp_s[:, c:c + QC])
            qq = (raw - m * csq_s[:, c:c + QC]) * rs
            for h in range(c // _L, (c + QC) // _L):
                q_s[h * B:(h + 1) * B, :] = qq[:, h * _L - c:(h + 1) * _L - c]

        P = {}

        def qk(i):
            g, b = pairs[i]
            qbg = q_s[pl.ds(g * rep * B + b, rep, stride=B), :].astype(bf16)
            s = jnp.concatenate([_dot(qbg, kt_r[i * NW + t]) for t in range(NW)], axis=1)
            mx = jnp.max(s, axis=-1, keepdims=True)
            p = jnp.exp(s - mx)
            P[i] = (p.astype(bf16), jnp.sum(p, axis=-1, keepdims=True))

        def pv(i):
            g, b = pairs[i]
            p, l = P.pop(i)
            o_s[pl.ds(g * rep * B + b, rep, stride=B), :] = _dot(p, v_v[b, g]) / l

        HC = D // 2
        acc = [x[:, :HC], x[:, HC:]]

        def wo(g):
            og = jnp.concatenate([o_s[h * B:(h + 1) * B, :] for h in range(g * rep, (g + 1) * rep)],
                                 axis=1).astype(bf16)
            for j in range(2):
                acc[j] = rowblocks(og, wo_v.at[:, pl.ds(j * HC, HC)], g * rep, (g + 1) * rep, acc[j])

        n = len(pairs)
        for i in range(LAG):
            qk(i)
        for i in range(n):
            pv(i)
            if i + LAG < n:
                qk(i + LAG)
            if i >= B + 3 and (i - 3) % B == 0 and (i - 3) // B - 1 < Hkv - 2:
                wo((i - 3) // B - 1)
        wo(Hkv - 2)
        wo(Hkv - 1)

        xb = [a.astype(bf16) for a in acc]
        xb_all = jnp.concatenate(xb, axis=1)
        x = xb_all.astype(f32)
        m, r, xc = _ln_stats(x)
        m2, r2, _ = _ln_stats(xc * r)
        ca = r * r2
        cb = (m * r + m2) * r2

        HP, H = {}, {}

        def w1_fin(f, raw):
            sl = slice(f * _L, (f + 1) * _L)
            H[f] = _gelu_tanh(raw * ca - cb * cs1_s[:, sl] + b1_s[:, sl]).astype(bf16)

        for f in range(NE):
            HP[f] = _dot(xb[0], w1_v[0:HC, f * _L:(f + 1) * _L])
        for f in range(NE):
            w1_fin(f, HP.pop(f) + _dot(xb[1], w1_v[HC:, f * _L:(f + 1) * _L]))

        xb2 = x + b2
        acc2 = [xb2[:, :CA * _L], xb2[:, CA * _L:(CA + CB) * _L], xb2[:, (CA + CB) * _L:]]

        def w2(f):
            hf = H.pop(f)
            for j, w_ref in enumerate((w2a_v, w2b_v, w2c_v)):
                acc2[j] = acc2[j] + _dot(hf, w_ref[f * _L:(f + 1) * _L, :])

        nxt = NE
        for f in range(NF):
            while nxt < NF and nxt <= f + LAG2 + (NE if f == 0 else 0):
                w1_fin(nxt, _dot(xb_all, w1_v[:, nxt * _L:(nxt + 1) * _L]))
                nxt += 1
            w2(f)
        o_ref[...] = jnp.concatenate(acc2, axis=1).astype(o_ref.dtype)

    any_spec = pl.BlockSpec(memory_space=pl.ANY)
    out = pl.pallas_call(
        kernel,
        out_shape=jax.ShapeDtypeStruct((B, D), A_x.dtype),
        in_specs=[any_spec] * 9,
        out_specs=pl.BlockSpec(memory_space=pltpu.VMEM),
        scratch_shapes=[
            pltpu.VMEM((B, D), bf16),
            pltpu.VMEM((F,), bf16),
            pltpu.VMEM((D,), bf16),
            pltpu.VMEM((D, HD), bf16),
            pltpu.VMEM((B, Hkv, W, Dh), bf16),
            pltpu.VMEM((B, Hkv, W, Dh), bf16),
            pltpu.VMEM((HD, D), bf16),
            pltpu.VMEM((D, F), bf16),
            pltpu.VMEM((F, CA * _L), bf16),
            pltpu.VMEM((F, CB * _L), bf16),
            pltpu.VMEM((F, CC * _L), bf16),
            pltpu.VMEM((B * Hkv * NW, Dh, _L), bf16),
            pltpu.VMEM((Hq * B, Dh), f32),
            pltpu.VMEM((Hq * B, Dh), f32),
            pltpu.VMEM((B, HD), f32),
            pltpu.VMEM((B, F), f32),
            pltpu.VMEM((B, F), f32),
            pltpu.VMEM((B, HD), f32),
            pltpu.SemaphoreType.DMA((NSEM,)),
        ],
        compiler_params=pltpu.CompilerParams(vmem_limit_bytes=100 * 1024 * 1024),
        name="fused",
    )(A_x.reshape(B, D), A_k_cache, A_v_cache, A_wq, A_wo, B_w1, B_b1, B_w2, B_b2)
    return out.reshape(B, Sq, D)
```

```python
import functools
import math

import jax
import jax.numpy as jnp
from jax import lax
import jax.experimental.pallas as pl
import jax.experimental.pallas.tpu as pltpu

_EPS = 1e-5
_L = 128
_LOG2E = 1.4426950408889634

_LA = 64
_LAE = 48
_SHIFT = 24
_LAG = 6
_LAG2 = 4
_NE = 8
_W2C = ((6, 16, ((20, 8), (8, 8))), (1, 64, ((28, 8),)), (1, 64, ((20, 8), (8, 8))))


def _gelu_tanh(x):
    c = 0.7978845608028654
    return 0.5 * x * (1.0 + jnp.tanh(c * (x + 0.044715 * (x * x * x))))


def _dot(a, b):
    return jnp.dot(a, b, preferred_element_type=jnp.float32)


def _layernorm(x):
    m = jnp.mean(x, axis=-1, keepdims=True)
    xc = x - m
    v = jnp.mean(xc * xc, axis=-1, keepdims=True)
    return xc * lax.rsqrt(v + _EPS)


def _blocksum(x):
    acc = x[:, :_L]
    for j in range(1, x.shape[1] // _L):
        acc = acc + x[:, j * _L:(j + 1) * _L]
    return acc


def _shift_partials(x_head):
    c = jnp.mean(x_head, axis=-1, keepdims=True)
    d = x_head - c
    return c, _blocksum(d), _blocksum(d * d)


def _shift_finish(parts, x_tail, n):
    c, s1, s2 = parts
    d = x_tail - c
    md = jnp.sum(s1 + _blocksum(d), axis=-1, keepdims=True) * (1.0 / n)
    ms = jnp.sum(s2 + _blocksum(d * d), axis=-1, keepdims=True) * (1.0 / n)
    v = jnp.maximum(ms - md * md, 0.0)
    return c + md, lax.rsqrt(v + _EPS)


def _pieces_2d(h, v, r0, nrows, c0, ncols, ns, pr, pc):
    per = nrows // ns
    assert per * ns == nrows and per % pr == 0 and ncols % pc == 0, (nrows, ns, pr)
    streams = [
        [(h.at[pl.ds(r, pr), pl.ds(c0 + c, pc)], v.at[pl.ds(r, pr), pl.ds(c, pc)])
         for r in range(r0 + s * per, r0 + (s + 1) * per, pr) for c in range(0, ncols, pc)]
        for s in range(ns)]
    return [p for tup in zip(*streams) for p in tup]


@jax.jit
def pallas_interleave_layers__sliding_block_cached__mixer_channel_mlp__decode_kernel(
    A_x: jax.Array,
    A_k_cache: jax.Array,
    A_v_cache: jax.Array,
    A_wq: jax.Array,
    A_wo: jax.Array,
    B_x: jax.Array,
    B_w1: jax.Array,
    B_b1: jax.Array,
    B_w2: jax.Array,
    B_b2: jax.Array,
):
    del B_x
    B, Sq, D = A_x.shape
    _, Hkv, Sk, Dh = A_k_cache.shape
    HD = A_wq.shape[1]
    Hq = HD // Dh
    F = B_w1.shape[1]
    W = min(4096, max(256, Sk // 4))
    rep = Hq // Hkv
    scale = Dh ** -0.5
    bf16, f32 = jnp.bfloat16, jnp.float32
    assert Sq == 1 and Dh == _L and B == 8 and rep == 8
    ND, NF, NW = D // _L, F // _L, W // _L
    NC = len(_W2C)
    c_off = [sum(c[0] for c in _W2C[:i]) for i in range(NC + 1)]
    assert c_off[NC] == ND
    n_tasks = 3 + B + sum(len(c[2]) for c in _W2C)
    pairs = [(g, b) for g in range(Hkv) for b in range(B)]
    QC = 8 * _L
    HC = D // 2

    def kernel(*refs):
        pl.run_scoped(functools.partial(body, *refs), pltpu.SemaphoreType.DMA((n_tasks,)))

    def body(x_h, k_h, v_h, wq_h, wo_h, w1_h, b1_h, w2_h, b2_h, o_ref,
             x_v, b1_v, b2_v, wq_v, k_v, v_v, wo_v, w1_v,
             kt_s, q_s, o_s, csq_s, cs1_s, b1_s, qp_s, *rest):
        w2_v, sems = rest[:-1], rest[-1]

        tasks = [([(x_h, x_v), (b1_h, b1_v), (b2_h, b2_v)]
                  + _pieces_2d(wq_h, wq_v, 0, D, 0, HD, 8, 8, HD // 2),
                  [x_v, b1_v, b2_v, wq_v])]
        for b in range(B):
            tasks.append(([(c_h.at[b, g, pl.ds(Sk - W + r, _L), :], c_v.at[b, g, pl.ds(r, _L), :])
                           for r in range(0, W, _L) for g in range(Hkv)
                           for c_h, c_v in ((k_h, k_v), (v_h, v_v))],
                          [k_v.at[b], v_v.at[b]]))
        tasks.append((_pieces_2d(wo_h, wo_v, 0, HD, 0, D, 8, 16, D), [wo_v]))
        tasks.append((_pieces_2d(w1_h, w1_v, 0, D, 0, F, 8, 8, F // 2), [w1_v]))
        for ci, (cw, pr, rsplit) in enumerate(_W2C):
            f0 = 0
            for nf, ns in rsplit:
                tasks.append((_pieces_2d(w2_h, w2_v[ci], f0 * _L, nf * _L, c_off[ci] * _L,
                                         cw * _L, ns, pr, cw * _L),
                              [w2_v[ci].at[pl.ds(f0 * _L, nf * _L)]]))
                f0 += nf
            assert f0 == NF
        assert len(tasks) == n_tasks
        nominal = [(s, d, t) for t, (ps, _) in enumerate(tasks) for s, d in ps]
        p0, p1 = nominal[0::2], nominal[1::2]
        flat = [e + (1,) for e in p1[:_SHIFT]]
        for i in range(len(p0)):
            flat.append(p0[i] + (0,))
            if i + _SHIFT < len(p1):
                flat.append(p1[i + _SHIFT] + (1,))
        assert len(flat) == len(nominal)
        ends = [1 + max(i for i, e in enumerate(flat) if e[2] == t) for t in range(n_tasks)]
        state = dict(issued=0, waited=0)

        def issue_until(n):
            t = state["waited"]
            if t < n_tasks:
                n = min(n, ends[t] + (_LA if t < 2 + B else _LAE))
            for s, d, t, prio in flat[state["issued"]:n]:
                pltpu.make_async_copy(s, d, sems.at[t]).start(priority=prio)
            state["issued"] = max(state["issued"], min(n, len(flat)))

        def pump(k):
            n, budget = state["issued"], k * 16 * 1024
            while n < len(flat) and budget > 0:
                budget -= math.prod(flat[n][1].shape)
                n += 1
            issue_until(n)

        def wait_next():
            t = state["waited"]
            issue_until(len(flat))
            assert state["issued"] >= ends[t]
            for buf in tasks[t][1]:
                pltpu.make_async_copy(buf, buf, sems.at[t]).wait()
            state["waited"] += 1

        def rowblocks(lhs, w_ref, k0, k1, acc=None):
            for k in range(k0, k1):
                r = _dot(lhs[:, (k - k0) * _L:(k - k0 + 1) * _L], w_ref[k * _L:(k + 1) * _L, :])
                acc = r if acc is None else acc + r
                pump(max(1, w_ref.shape[1] // QC))
            return acc

        def head_rows(g, b):
            return pl.ds(g * rep * B + b, rep, stride=B)

        def store_heads(q, c):
            for j in range(QC // _L):
                h = c // _L + j
                q_s[h * B:(h + 1) * B, :] = q[:, j * _L:(j + 1) * _L]

        def load_heads(h0, h1):
            return jnp.concatenate([o_s[h * B:(h + 1) * B, :] for h in range(h0, h1)],
                                   axis=1).astype(bf16)

        ones = jnp.ones((B, D), bf16)

        wait_next()
        x = x_v[...].astype(f32)
        b1_s[...] = jnp.broadcast_to(b1_v[...].astype(f32).reshape(1, F), (B, F))
        b2 = jnp.broadcast_to(b2_v[...].astype(f32).reshape(1, D), (B, D))
        lhs = jnp.concatenate([_layernorm(x).astype(bf16), ones], axis=0)
        for c in range(0, HD, QC):
            res = rowblocks(lhs, wq_v.at[:, pl.ds(c, QC)], 0, ND)
            csq_s[:, c:c + QC] = res[B:]
            store_heads(res[:B] * scale, c)

        for b in range(B):
            wait_next()
            for g in range(Hkv):
                qbg = q_s[head_rows(g, b), :].astype(bf16)
                ss = []
                for t in range(NW):
                    kt = k_v[b, g, t * _L:(t + 1) * _L, :].T
                    kt_s[(g * B + b) * NW + t] = kt
                    ss.append(_dot(qbg, kt))
                    pump(2)
                s = jnp.concatenate(ss, axis=1)
                p = jnp.exp(s - jnp.max(s, axis=-1, keepdims=True))
                l = jnp.sum(p, axis=-1, keepdims=True)
                o_s[head_rows(g, b), :] = _dot(p.astype(bf16), v_v[b, g]) / l

        oc = load_heads(0, Hq)
        wait_next()
        x = rowblocks(oc, wo_v, 0, Hq, x).astype(bf16).astype(f32)
        lhs = jnp.concatenate([_layernorm(_layernorm(x)).astype(bf16), ones], axis=0)

        wait_next()
        hs = []
        for f in range(NF):
            res = _dot(lhs, w1_v[:, f * _L:(f + 1) * _L])
            cs1_s[:, f * _L:(f + 1) * _L] = res[B:]
            hs.append(_gelu_tanh(res[:B] + b1_s[:, f * _L:(f + 1) * _L]).astype(bf16))
            pump(1)
        hc = jnp.concatenate(hs, axis=1)
        xb2 = x + b2

        xs = []
        for ci, (cw, _, rsplit) in enumerate(_W2C):
            acc = xb2[:, c_off[ci] * _L:c_off[ci + 1] * _L]
            if ci == NC - 1:
                parts = _shift_partials(jnp.concatenate(xs, axis=1).astype(f32))
            f0 = 0
            for nf, _ in rsplit:
                wait_next()
                hpart = hc[:, f0 * _L:(f0 + nf) * _L]
                if cw == 1:
                    acc = acc + _dot(hpart, w2_v[ci][f0 * _L:(f0 + nf) * _L, :])
                else:
                    acc = rowblocks(hpart, w2_v[ci], f0, f0 + nf, acc)
                f0 += nf
            xs.append(acc.astype(bf16))
            if ci < NC - 1:
                for c in range(0, HD, QC):
                    qp_s[:, c:c + QC] = rowblocks(
                        xs[ci], wq_v.at[:, pl.ds(c, QC)], c_off[ci], c_off[ci + 1],
                        qp_s[:, c:c + QC] if ci else None)
        assert state["waited"] == n_tasks and state["issued"] == len(flat)

        x = jnp.concatenate(xs, axis=1).astype(f32)
        m, r = _shift_finish(parts, xs[-1].astype(f32), D)
        rs = jnp.broadcast_to(r * (scale * _LOG2E), (B, _L))
        rsb = [jnp.broadcast_to(rs[b:b + 1, :], (rep, _L)) for b in range(B)]
        for c in range(0, HD, QC):
            raw = rowblocks(xs[-1], wq_v.at[:, pl.ds(c, QC)], c_off[NC - 1], ND,
                            qp_s[:, c:c + QC])
            store_heads(raw - m * csq_s[:, c:c + QC], c)

        probs = {}

        def qk(i):
            g, b = pairs[i]
            qbg = q_s[head_rows(g, b), :].astype(bf16)
            s = jnp.concatenate([_dot(qbg, kt_s[i * NW + t]) for t in range(NW)], axis=1)
            mx = jnp.max(s, axis=-1, keepdims=True)
            p = jnp.exp2((s - mx) * jnp.concatenate([rsb[b]] * NW, axis=1))
            probs[i] = (p.astype(bf16), jnp.sum(p, axis=-1, keepdims=True))

        def pv(i):
            g, b = pairs[i]
            p, l = probs.pop(i)
            o_s[head_rows(g, b), :] = _dot(p, v_v[b, g]) / l

        acc = [x[:, :HC], x[:, HC:]]

        def wo(g):
            og = load_heads(g * rep, (g + 1) * rep)
            for j in range(2):
                acc[j] = rowblocks(og, wo_v.at[:, pl.ds(j * HC, HC)], g * rep, (g + 1) * rep,
                                   acc[j])

        n = len(pairs)
        for i in range(_LAG):
            qk(i)
        for i in range(n):
            pv(i)
            if i + _LAG < n:
                qk(i + _LAG)
            g_done, off = divmod(i - 3, B)
            if off == 0 and 1 <= g_done <= Hkv - 2:
                wo(g_done - 1)
        wo(Hkv - 2)
        wo(Hkv - 1)

        xb = [a.astype(bf16) for a in acc]
        xb_all = jnp.concatenate(xb, axis=1)
        x = xb_all.astype(f32)
        m, r = _shift_finish(_shift_partials(x[:, :HC]), x[:, HC:], D)
        u = (x - m) * r
        m2 = jnp.mean(u, axis=-1, keepdims=True)
        v2 = jnp.maximum(jnp.mean(u * u, axis=-1, keepdims=True) - m2 * m2, 0.0)
        r2 = lax.rsqrt(v2 + _EPS)
        ca = r * r2
        cb = (m * r + m2) * r2

        hid = {}

        def w1_fin(f, *raws):
            sl = slice(f * _L, (f + 1) * _L)
            pre = b1_s[:, sl] - cb * cs1_s[:, sl]
            for raw in raws:
                pre = pre + raw * ca
            hid[f] = _gelu_tanh(pre).astype(bf16)

        early = [_dot(xb[0], w1_v[0:HC, f * _L:(f + 1) * _L]) for f in range(_NE)]
        for f in range(_NE):
            w1_fin(f, early[f], _dot(xb[1], w1_v[HC:, f * _L:(f + 1) * _L]))

        xb2 = x + b2
        acc2 = [xb2[:, c_off[ci] * _L:c_off[ci + 1] * _L] for ci in range(NC)]
        nxt = _NE
        for f in range(NF):
            while nxt < NF and nxt <= f + _LAG2 + (_NE if f == 0 else 0):
                w1_fin(nxt, _dot(xb_all, w1_v[:, nxt * _L:(nxt + 1) * _L]))
                nxt += 1
            hf = hid.pop(f)
            for ci in range(NC):
                acc2[ci] = acc2[ci] + _dot(hf, w2_v[ci][f * _L:(f + 1) * _L, :])
        o_ref[...] = jnp.concatenate(acc2, axis=1).astype(o_ref.dtype)

    out = pl.pallas_call(
        kernel,
        out_shape=jax.ShapeDtypeStruct((B, D), A_x.dtype),
        in_specs=[pl.BlockSpec(memory_space=pl.ANY)] * 9,
        out_specs=pl.BlockSpec(memory_space=pltpu.VMEM),
        scratch_shapes=[
            pltpu.VMEM((B, D), bf16),
            pltpu.VMEM((F,), bf16),
            pltpu.VMEM((D,), bf16),
            pltpu.VMEM((D, HD), bf16),
            pltpu.VMEM((B, Hkv, W, Dh), bf16),
            pltpu.VMEM((B, Hkv, W, Dh), bf16),
            pltpu.VMEM((HD, D), bf16),
            pltpu.VMEM((D, F), bf16),
            pltpu.VMEM((B * Hkv * NW, Dh, _L), bf16),
            pltpu.VMEM((Hq * B, Dh), f32),
            pltpu.VMEM((Hq * B, Dh), f32),
            pltpu.VMEM((B, HD), f32),
            pltpu.VMEM((B, F), f32),
            pltpu.VMEM((B, F), f32),
            pltpu.VMEM((B, HD), f32),
        ] + [pltpu.VMEM((F, c[0] * _L), bf16) for c in _W2C],
        compiler_params=pltpu.CompilerParams(vmem_limit_bytes=100 * 1024 * 1024),
        name="fused_decode_layers",
    )(A_x.reshape(B, D), A_k_cache, A_v_cache, A_wq, A_wo, B_w1, B_b1, B_w2, B_b2)
    return out.reshape(B, Sq, D)
```

```python
import functools
import math

import jax
import jax.numpy as jnp
from jax import lax
import jax.experimental.pallas as pl
import jax.experimental.pallas.tpu as pltpu

_EPS = 1e-5
_L = 128
_LOG2E = 1.4426950408889634

_NS = 8
_PT = 16
_PHASE = dict(q=5, kv=5, o=5, w1=13)
_SUB = dict(q=2, o=4, w1=2)
_LA = 64
_LAE = 48
_SHIFT = 20
_LAG = 6
_LAG2 = 4
_NE = 8
_W2BUF = ((0, 6), (6, 7), (7, 8))
_W2T = ((0, 24, 0, 6, 8, 32), (24, 4, 0, 6, 8, 32), (0, 28, 6, 1, 4, 128),
        (0, 20, 7, 1, 4, 128), (20, 8, 7, 1, 8, 128))


def _gelu_tanh(x):
    c = 0.7978845608028654
    return 0.5 * x * (1.0 + jnp.tanh(c * (x + 0.044715 * (x * x * x))))


def _dot(a, b):
    return jnp.dot(a, b, preferred_element_type=jnp.float32)


def _layernorm(x):
    m = jnp.mean(x, axis=-1, keepdims=True)
    xc = x - m
    v = jnp.mean(xc * xc, axis=-1, keepdims=True)
    return xc * lax.rsqrt(v + _EPS)


def _blocksum(x):
    acc = x[:, :_L]
    for j in range(1, x.shape[1] // _L):
        acc = acc + x[:, j * _L:(j + 1) * _L]
    return acc


def _shift_partials(x_head):
    c = jnp.mean(x_head, axis=-1, keepdims=True)
    d = x_head - c
    return c, _blocksum(d), _blocksum(d * d)


def _shift_finish(parts, x_tail, n):
    c, s1, s2 = parts
    d = x_tail - c
    md = jnp.sum(s1 + _blocksum(d), axis=-1, keepdims=True) * (1.0 / n)
    ms = jnp.sum(s2 + _blocksum(d * d), axis=-1, keepdims=True) * (1.0 / n)
    v = jnp.maximum(ms - md * md, 0.0)
    return c + md, lax.rsqrt(v + _EPS)


def _rect_streams(h, v, r0, nrows, c0, ncols, ns, pr):
    per = nrows // ns
    assert per * ns == nrows and per % pr == 0 and v.shape[1] == ncols, (nrows, ns, pr)
    return [[[(h.at[pl.ds(r, pr), pl.ds(c0, ncols)], v.at[pl.ds(r, pr), :])]
             for r in range(r0 + s * per, r0 + (s + 1) * per, pr)] for s in range(ns)]


def _flat_slices(nb, t0, nt):
    r0, c0 = divmod(t0, nb)
    r1, c1 = divmod(t0 + nt, nb)
    if r0 == r1:
        return [(pl.ds(r0 * 8, 8), pl.ds(c0 * _L, (c1 - c0) * _L))]
    out = []
    cuts = sorted({0, c0, c1, nb})
    for a, b in zip(cuts[:-1], cuts[1:]):
        top = r0 if a >= c0 else r0 + 1
        bot = r1 + 1 if b <= c1 else r1
        if bot > top:
            out.append((pl.ds(top * 8, (bot - top) * 8), pl.ds(a * _L, (b - a) * _L)))
    return out


def _flat_streams(h, v, ns, phase):
    nb = h.shape[1] // _L
    nt = (h.shape[0] // 8) * nb
    assert nt % (ns * _PT) == 0 and 0 <= phase < _PT
    per = nt // (ns * _PT)
    cuts = [0] + list(range(phase + _PT, nt, _PT)) + [nt]
    assert len(cuts) == ns * per + 1
    pieces = [[(h.at[sl], v.at[sl]) for sl in _flat_slices(nb, a, b - a)]
              for a, b in zip(cuts[:-1], cuts[1:])]
    return ([pieces[s * per:(s + 1) * per] for s in range(ns)],
            [(cuts[s * per], cuts[(s + 1) * per]) for s in range(ns)])


@jax.jit
def pallas_interleave_layers__sliding_block_cached__mixer_channel_mlp__decode_kernel(
    A_x: jax.Array,
    A_k_cache: jax.Array,
    A_v_cache: jax.Array,
    A_wq: jax.Array,
    A_wo: jax.Array,
    B_x: jax.Array,
    B_w1: jax.Array,
    B_b1: jax.Array,
    B_w2: jax.Array,
    B_b2: jax.Array,
):
    del B_x
    B, Sq, D = A_x.shape
    _, Hkv, Sk, Dh = A_k_cache.shape
    HD = A_wq.shape[1]
    Hq = HD // Dh
    F = B_w1.shape[1]
    W = min(4096, max(256, Sk // 4))
    rep = Hq // Hkv
    scale = Dh ** -0.5
    bf16, f32 = jnp.bfloat16, jnp.float32
    assert Sq == 1 and Dh == _L and B == 8 and rep == 8 and F <= HD
    ND, NF, NW = D // _L, F // _L, W // _L
    n_tasks = _SUB["q"] + B * Hkv + _SUB["o"] + _SUB["w1"] + len(_W2T)
    pairs = [(g, b) for g in range(Hkv) for b in range(B)]
    QC = 8 * _L
    HC = D // 2

    def kernel(*refs):
        pl.run_scoped(functools.partial(body, *refs), pltpu.SemaphoreType.DMA((n_tasks,)))

    def body(x_h, k_h, v_h, wq_h, wo_h, w1_h, b1_h, w2_h, b2_h, o_ref,
             x_v, b1_v, b2_v, wq_v, k_v, v_v, wo_v, w1_v,
             kt_s, q_s, o_s, csq_s, cs1_s, b1_s, part_s, *rest):
        w2_v, sems = rest[:-1], rest[-1]

        nominal, waits, group_of = [], [], []

        def add_group(labelled_streams, task_waits, head=()):
            g, t0 = (group_of[-1] + 1 if group_of else 0), len(waits)
            nominal.extend((p, t0) for p in head)
            for tup in zip(*[s for s, _ in labelled_streams]):
                nominal.extend((p, t0 + lab) for p, (_, lab) in zip(tup, labelled_streams))
            waits.extend(task_waits)
            group_of.extend([g] * len(task_waits))

        def add_flat(h, v, phase, nsub, head=(), head_waits=()):
            streams, spans = _flat_streams(h, v, _NS, phase)
            k = _NS // nsub
            tw = [[v.at[sl] for sl in _flat_slices(
                h.shape[1] // _L, spans[i * k][0], spans[(i + 1) * k - 1][1] - spans[i * k][0])]
                for i in range(nsub)]
            tw[0] = list(head_waits) + tw[0]
            add_group([(s, i // k) for i, s in enumerate(streams)], tw, head)

        add_flat(wq_h, wq_v, _PHASE["q"], _SUB["q"],
                 head=[[(x_h, x_v)], [(b1_h, b1_v), (b2_h, b2_v)]],
                 head_waits=[x_v, b1_v, b2_v])
        for b in range(B):
            add_group([(_flat_streams(c_h.at[b, g, pl.ds(Sk - W, W), :], c_v.at[b, g], 1,
                                      _PHASE["kv"])[0][0], g)
                       for g in range(Hkv) for c_h, c_v in ((k_h, k_v), (v_h, v_v))],
                      [[k_v.at[b, g], v_v.at[b, g]] for g in range(Hkv)])
        add_flat(wo_h, wo_v, _PHASE["o"], _SUB["o"])
        add_flat(w1_h, w1_v, _PHASE["w1"], _SUB["w1"])
        late_group = group_of[-1]
        for f0, nf, c0, nc, ns, pr in _W2T:
            buf = w2_v[_W2BUF.index((c0, c0 + nc))]
            add_group([(s, 0) for s in _rect_streams(w2_h, buf, f0 * _L, nf * _L, c0 * _L,
                                                     nc * _L, ns, pr)],
                      [[buf.at[pl.ds(f0 * _L, nf * _L), :]]])
        assert len(waits) == n_tasks
        n_groups = group_of[-1] + 1
        p0, p1 = nominal[0::2], nominal[1::2]
        flat = [e + (1,) for e in p1[:_SHIFT]]
        for i in range(len(p0)):
            flat.append(p0[i] + (0,))
            if i + _SHIFT < len(p1):
                flat.append(p1[i + _SHIFT] + (1,))
        assert len(flat) == len(nominal)
        gend = [1 + max(i for i, e in enumerate(flat) if group_of[e[1]] == g)
                for g in range(n_groups)]
        state = dict(issued=0, waited=0, group=0)

        def issue_until(n):
            g = state["group"]
            if g < n_groups:
                lim, budget = gend[g], (_LA if g < late_group else _LAE)
                while lim < len(flat) and budget >= len(flat[lim][0]):
                    budget -= len(flat[lim][0])
                    lim += 1
                n = min(n, lim)
            for piece, t, prio in flat[state["issued"]:n]:
                for s, d in piece:
                    pltpu.make_async_copy(s, d, sems.at[t]).start(priority=prio)
            state["issued"] = max(state["issued"], min(n, len(flat)))

        def pump(k):
            n, budget = state["issued"], k * 16 * 1024
            while n < len(flat) and budget > 0:
                budget -= sum(math.prod(d.shape) for _, d in flat[n][0])
                n += 1
            issue_until(n)

        def wait_next():
            t = state["waited"]
            if group_of[t] == state["group"]:
                issue_until(len(flat))
                state["group"] += 1
            assert state["issued"] >= gend[group_of[t]]
            for buf in waits[t]:
                pltpu.make_async_copy(buf, buf, sems.at[t]).wait()
            state["waited"] += 1

        def rowblocks(lhs, w_ref, k0, k1, acc=None):
            for k in range(k0, k1):
                r = _dot(lhs[:, (k - k0) * _L:(k - k0 + 1) * _L], w_ref[k * _L:(k + 1) * _L, :])
                acc = r if acc is None else acc + r
                pump(max(1, w_ref.shape[1] // QC))
            return acc

        def head_rows(g, b):
            return pl.ds(g * rep * B + b, rep, stride=B)

        def store_heads(q, c):
            for j in range(QC // _L):
                h = c // _L + j
                q_s[h * B:(h + 1) * B, :] = q[:, j * _L:(j + 1) * _L]

        def load_heads(h0, h1):
            return jnp.concatenate([o_s[h * B:(h + 1) * B, :] for h in range(h0, h1)],
                                   axis=1).astype(bf16)

        ones = jnp.ones((B, D), bf16)

        kq = ND // _SUB["q"]
        for i in range(_SUB["q"]):
            wait_next()
            if i == 0:
                x = x_v[...].astype(f32)
                b1_s[...] = jnp.broadcast_to(b1_v[...].astype(f32).reshape(1, F), (B, F))
                b2 = jnp.broadcast_to(b2_v[...].astype(f32).reshape(1, D), (B, D))
                lhs = jnp.concatenate([_layernorm(x).astype(bf16), ones], axis=0)
            for c in range(0, HD, QC):
                prev = None if i == 0 else jnp.concatenate(
                    [part_s[:, c:c + QC], csq_s[:, c:c + QC]], axis=0)
                res = rowblocks(lhs[:, i * kq * _L:(i + 1) * kq * _L], wq_v.at[:, pl.ds(c, QC)],
                                i * kq, (i + 1) * kq, prev)
                csq_s[:, c:c + QC] = res[B:]
                if i == _SUB["q"] - 1:
                    store_heads(res[:B] * scale, c)
                else:
                    part_s[:, c:c + QC] = res[:B]

        for b in range(B):
            for g in range(Hkv):
                wait_next()
                qbg = q_s[head_rows(g, b), :].astype(bf16)
                ss = []
                for t in range(NW):
                    kt = k_v[b, g, t * _L:(t + 1) * _L, :].T
                    kt_s[(g * B + b) * NW + t] = kt
                    ss.append(_dot(qbg, kt))
                    pump(2)
                s = jnp.concatenate(ss, axis=1)
                p = jnp.exp(s - jnp.max(s, axis=-1, keepdims=True))
                l = jnp.sum(p, axis=-1, keepdims=True)
                o_s[head_rows(g, b), :] = _dot(p.astype(bf16), v_v[b, g]) / l

        ko = Hq // _SUB["o"]
        for i in range(_SUB["o"]):
            wait_next()
            x = rowblocks(load_heads(i * ko, (i + 1) * ko), wo_v, i * ko, (i + 1) * ko, x)
        x = x.astype(bf16).astype(f32)
        lhs = jnp.concatenate([_layernorm(_layernorm(x)).astype(bf16), ones], axis=0)

        k1 = D // _SUB["w1"]
        hs = []
        for i in range(_SUB["w1"]):
            wait_next()
            for f in range(NF):
                sl = slice(f * _L, (f + 1) * _L)
                prev = ([b1_s[:, sl], jnp.zeros((B, _L), f32)] if i == 0
                        else [part_s[:, sl], cs1_s[:, sl]])
                res = jnp.concatenate(prev, axis=0) + _dot(
                    lhs[:, i * k1:(i + 1) * k1], w1_v[i * k1:(i + 1) * k1, sl])
                cs1_s[:, sl] = res[B:]
                if i == _SUB["w1"] - 1:
                    hs.append(_gelu_tanh(res[:B]).astype(bf16))
                else:
                    part_s[:, sl] = res[:B]
                if f % _SUB["w1"] == 0:
                    pump(1)
        hc = jnp.concatenate(hs, axis=1)
        xb2 = x + b2

        accs = [xb2[:, lo * _L:hi * _L] for lo, hi in _W2BUF]
        done = [0] * len(_W2BUF)
        xs = []
        for ti, (f0, nf, c0, nc, _, _) in enumerate(_W2T):
            last = ti == len(_W2T) - 1
            if last:
                parts = _shift_partials(jnp.concatenate(xs, axis=1).astype(f32))
            wait_next()
            bi = _W2BUF.index((c0, c0 + nc))
            hpart = hc[:, f0 * _L:(f0 + nf) * _L]
            if nc == 1:
                accs[bi] = accs[bi] + _dot(hpart, w2_v[bi][f0 * _L:(f0 + nf) * _L, :])
            else:
                accs[bi] = rowblocks(hpart, w2_v[bi], f0, f0 + nf, accs[bi])
            done[bi] += nf
            if done[bi] == NF:
                assert bi == len(xs)
                xs.append(accs[bi].astype(bf16))
                if not last:
                    for c in range(0, HD, QC):
                        part_s[:, c:c + QC] = rowblocks(
                            xs[bi], wq_v.at[:, pl.ds(c, QC)], c0, c0 + nc,
                            part_s[:, c:c + QC] if bi else None)
        assert len(xs) == len(_W2BUF) and _W2BUF[-1] == (c0, ND)
        assert state["waited"] == n_tasks and state["issued"] == len(flat)

        x = jnp.concatenate(xs, axis=1).astype(f32)
        m, r = _shift_finish(parts, xs[-1].astype(f32), D)
        rs = jnp.broadcast_to(r * (scale * _LOG2E), (B, _L))
        rsb = [jnp.broadcast_to(rs[b:b + 1, :], (rep, _L)) for b in range(B)]
        for c in range(0, HD, QC):
            raw = rowblocks(xs[-1], wq_v.at[:, pl.ds(c, QC)], c0, ND, part_s[:, c:c + QC])
            store_heads(raw - m * csq_s[:, c:c + QC], c)

        probs = {}

        def qk(i):
            g, b = pairs[i]
            qbg = q_s[head_rows(g, b), :].astype(bf16)
            s = jnp.concatenate([_dot(qbg, kt_s[i * NW + t]) for t in range(NW)], axis=1)
            mx = jnp.max(s, axis=-1, keepdims=True)
            p = jnp.exp2((s - mx) * jnp.concatenate([rsb[b]] * NW, axis=1))
            probs[i] = (p.astype(bf16), jnp.sum(p, axis=-1, keepdims=True))

        def pv(i):
            g, b = pairs[i]
            p, l = probs.pop(i)
            o_s[head_rows(g, b), :] = _dot(p, v_v[b, g]) / l

        acc = [x[:, :HC], x[:, HC:]]

        def wo(g):
            og = load_heads(g * rep, (g + 1) * rep)
            for j in range(2):
                acc[j] = rowblocks(og, wo_v.at[:, pl.ds(j * HC, HC)], g * rep, (g + 1) * rep,
                                   acc[j])

        n = len(pairs)
        for i in range(_LAG):
            qk(i)
        for i in range(n):
            pv(i)
            if i + _LAG < n:
                qk(i + _LAG)
            g_next, off = divmod(i - 3, B)
            if off == 0 and 1 <= g_next <= Hkv - 2:
                wo(g_next - 1)
        wo(Hkv - 2)
        wo(Hkv - 1)

        xb = [a.astype(bf16) for a in acc]
        xb_all = jnp.concatenate(xb, axis=1)
        x = xb_all.astype(f32)
        m, r = _shift_finish(_shift_partials(x[:, :HC]), x[:, HC:], D)
        u = (x - m) * r
        m2 = jnp.mean(u, axis=-1, keepdims=True)
        v2 = jnp.maximum(jnp.mean(u * u, axis=-1, keepdims=True) - m2 * m2, 0.0)
        r2 = lax.rsqrt(v2 + _EPS)
        ca = r * r2
        cb = (m * r + m2) * r2

        hid = {}

        def w1_fin(f, *raws):
            sl = slice(f * _L, (f + 1) * _L)
            pre = b1_s[:, sl] - cb * cs1_s[:, sl]
            for raw in raws:
                pre = pre + raw * ca
            hid[f] = _gelu_tanh(pre).astype(bf16)

        early = [_dot(xb[0], w1_v[0:HC, f * _L:(f + 1) * _L]) for f in range(_NE)]
        for f in range(_NE):
            w1_fin(f, early[f], _dot(xb[1], w1_v[HC:, f * _L:(f + 1) * _L]))

        xb2 = x + b2
        acc2 = [xb2[:, lo * _L:hi * _L] for lo, hi in _W2BUF]
        nxt = _NE
        for f in range(NF):
            while nxt < NF and nxt <= f + _LAG2 + (_NE if f == 0 else 0):
                w1_fin(nxt, _dot(xb_all, w1_v[:, nxt * _L:(nxt + 1) * _L]))
                nxt += 1
            hf = hid.pop(f)
            for bi in range(len(_W2BUF)):
                acc2[bi] = acc2[bi] + _dot(hf, w2_v[bi][f * _L:(f + 1) * _L, :])
        o_ref[...] = jnp.concatenate(acc2, axis=1).astype(o_ref.dtype)

    out = pl.pallas_call(
        kernel,
        out_shape=jax.ShapeDtypeStruct((B, D), A_x.dtype),
        in_specs=[pl.BlockSpec(memory_space=pl.ANY)] * 9,
        out_specs=pl.BlockSpec(memory_space=pltpu.VMEM),
        scratch_shapes=[
            pltpu.VMEM((B, D), bf16),
            pltpu.VMEM((F,), bf16),
            pltpu.VMEM((D,), bf16),
            pltpu.VMEM((D, HD), bf16),
            pltpu.VMEM((B, Hkv, W, Dh), bf16),
            pltpu.VMEM((B, Hkv, W, Dh), bf16),
            pltpu.VMEM((HD, D), bf16),
            pltpu.VMEM((D, F), bf16),
            pltpu.VMEM((B * Hkv * NW, Dh, _L), bf16),
            pltpu.VMEM((Hq * B, Dh), f32),
            pltpu.VMEM((Hq * B, Dh), f32),
            pltpu.VMEM((B, HD), f32),
            pltpu.VMEM((B, F), f32),
            pltpu.VMEM((B, F), f32),
            pltpu.VMEM((B, HD), f32),
        ] + [pltpu.VMEM((F, (hi - lo) * _L), bf16) for lo, hi in _W2BUF],
        compiler_params=pltpu.CompilerParams(vmem_limit_bytes=100 * 1024 * 1024),
        name="fused_decode_layers",
    )(A_x.reshape(B, D), A_k_cache, A_v_cache, A_wq, A_wo, B_w1, B_b1, B_w2, B_b2)
    return out.reshape(B, Sq, D)
```
